```python
import os as _os
_os.environ.setdefault("JAX_PLATFORMS", "cpu")
import jax
import jax.numpy as jnp

def _softmax(x, axis=-1):
    return jax.nn.softmax(x, axis=axis)
def _gelu(x):
    return jax.nn.gelu(x, approximate=True)
def _silu(x):
    return jax.nn.silu(x)
def _sigmoid(x):
    return jax.nn.sigmoid(x)
def _layernorm(x, axis=-1, eps=1e-5):
    m = jnp.mean(x, axis=axis, keepdims=True)
    v = jnp.var(x, axis=axis, keepdims=True)
    return (x - m) / jnp.sqrt(v + eps)
def _scatter_add(tgt, idx, src, axis=0):
    return tgt.at[idx].add(src)
def _segment_sum(src, seg, n):
    return jax.ops.segment_sum(src, seg, n)
class _Rng:
    def __init__(self, key):
        self._k = key
    def _next(self):
        self._k, sub = jax.random.split(self._k)
        return sub
    def normal(self, shape):
        return jax.random.normal(self._next(), shape, dtype=jnp.bfloat16)
    def randint(self, lo, hi, shape):
        return jax.random.randint(self._next(), shape, lo, hi, dtype=jnp.int32)
    def uniform(self, shape, lo=0.0, hi=1.0):
        return jax.random.uniform(self._next(), shape, jnp.bfloat16, lo, hi)
    def permutation(self, n):
        return jax.random.permutation(self._next(), n)


kernel_name = 'interleave_layers__linear_attn_block__mha_block__prompt'

def setup_inputs():
    _rng = _Rng(jax.random.key(int.from_bytes(__import__("os").urandom(4), "little")))
    _w = (lambda a: (lambda t: t.astype(jnp.bfloat16) if jnp.issubdtype(t.dtype, jnp.floating) else t)(jnp.asarray(a)))
    def _A_setup():
        B, S, D = 1, 2048, 640
        return {
            "x": _w((lambda *s: _rng.normal(s) * 0.05)(B, S, D)),
            "wqkv": _w((lambda *s: _rng.normal(s) * 0.1)(D, 3 * D)),
            "wo": _w((lambda *s: _rng.normal(s) * 0.05)(D, D)),
        }
    _A_in = _A_setup()

    def _B_setup():
        B, S, D, H = 1, 2048, 640, 32
        return {
            "x": _w((lambda *s: _rng.normal(s) * 0.05)(B, S, D)),
            "wqkv": _w((lambda *s: _rng.normal(s) * 0.1)(D, 3 * D)),
            "wo": _w((lambda *s: _rng.normal(s) * 0.05)(D, D)),
        }
    _B_in = _B_setup()

    return {
        "A_x": _A_in["x"],
        "A_wqkv": _A_in["wqkv"],
        "A_wo": _A_in["wo"],
        "B_x": _B_in["x"],
        "B_wqkv": _B_in["wqkv"],
        "B_wo": _B_in["wo"],
    }

def reference(A_x, A_wqkv, A_wo, B_x, B_wqkv, B_wo):
    def _A_ref(x, wqkv, wo):
        B, S, D = x.shape
        H = 32; Dh = D // H
        qkv = (lambda x, *d: x.transpose(*d))((x @ wqkv).reshape(B, S, 3, H, Dh), 2, 0, 3, 1, 4)
        q, k, v = qkv[0], qkv[1], qkv[2]
        phi = lambda t: jnp.where(t > 0, t + 1, jnp.exp(t)) + 1e-6
        pq, pk = phi(q), phi(k)
        kv = jnp.einsum("bhsd,bhse->bhde", pk, v)
        z = jnp.einsum("bhsd->bhd", pk)
        num = jnp.einsum("bhqd,bhde->bhqe", pq, kv)
        den = jnp.einsum("bhqd,bhd->bhq", pq, z)[..., None] + 1e-6
        o = num / den
        return (lambda x, *d: x.transpose(*d))(o, 0, 2, 1, 3).reshape(B, S, D) @ wo

    def _B_ref(x, wqkv, wo):
        B, S, D = x.shape
        H = 32
        Dh = D // H
        qkv = (lambda x, *d: x.transpose(*d))((x @ wqkv).reshape(B, S, 3, H, Dh), 2, 0, 3, 1, 4)
        q, k, v = qkv[0], qkv[1], qkv[2]
        scores = jnp.einsum("bhqd,bhkd->bhqk", q, k) * (Dh ** -0.5)
        p = _softmax(scores, axis=-1)
        o = jnp.einsum("bhqk,bhkd->bhqd", p, v)
        return (lambda x, *d: x.transpose(*d))(o, 0, 2, 1, 3).reshape(B, S, D) @ wo

    x = A_x
    x = x + _A_ref(_layernorm(x, axis=-1), A_wqkv, A_wo)
    x = x + _B_ref(_layernorm(x, axis=-1), B_wqkv, B_wo)
    x = x + _A_ref(_layernorm(x, axis=-1), A_wqkv, A_wo)
    x = x + _B_ref(_layernorm(x, axis=-1), B_wqkv, B_wo)
    return x
```

```python
import functools

import jax
import jax.numpy as jnp
import numpy as np
from jax import lax
import jax.experimental.pallas as pl
import jax.experimental.pallas.tpu as pltpu

S = 2048
D = 640
H = 32
DH = D // H
T = 512
NQ = 256
CH = 128
G = 8
VR = 24
NW = 6
F32 = jnp.float32
BF16 = jnp.bfloat16

BANDS = ((0, 144), (112, 272), (240, 400), (368, 528), (496, 640))
BAND_MAX = 160
WIN = (0, 120, 240, 360, 480, 512)


def _layernorm_t(x):
    m = jnp.sum(x, axis=0, keepdims=True) * (1.0 / D)
    xc = x - m
    v = jnp.sum(xc * xc, axis=0, keepdims=True) * (1.0 / D)
    return (xc * lax.rsqrt(v + 1e-5)).astype(BF16)


def _head_of(i):
    return (i * 3277) >> 16


def _phi(t):
    return jnp.where(t > 0, t + 1.0, jnp.exp(t)) + 1e-6


def _dot(a, b):
    return lax.dot_general(a, b, (((1,), (0,)), ((), ())),
                           preferred_element_type=F32)


def _dot_nt(a, b):
    return lax.dot_general(a, b, (((1,), (1,)), ((), ())),
                           preferred_element_type=F32)


def _transpose_into(dst, src):
    for j in range(src.shape[1] // 128):
        dst[j * 128:(j + 1) * 128, :] = (
            src[:, j * 128:(j + 1) * 128].astype(F32).T.astype(BF16))


def _kernel(x_hbm, awqkv_hbm, awo_hbm, bwqkv_hbm, bwo_hbm, o_hbm,
            xio, awqkv_v, awo_v, bwqkv_v, bwo_v, sems,
            xt, wa, woa, wb, wob, pq, pk, va, kvz, qw, kw, vw, ot,
            s_a, s_b, m_ref):
    nch = S // T

    def x_in(c):
        rows = pl.ds(pl.multiple_of(c * T, T), T)
        return pltpu.make_async_copy(x_hbm.at[rows], xio.at[rows], sems.at[c])

    def x_out(c):
        rows = pl.ds(pl.multiple_of(c * T, T), T)
        return pltpu.make_async_copy(xio.at[rows], o_hbm.at[rows], sems.at[c])

    w_in = [pltpu.make_async_copy(src, dst, sems.at[nch + i])
            for i, (src, dst) in enumerate((
                (awqkv_hbm, awqkv_v), (awo_hbm, awo_v),
                (bwqkv_hbm, bwqkv_v), (bwo_hbm, bwo_v)))]

    w_in[0].start()
    x_in(0).start()
    w_in[0].wait()
    for c in range(1, nch):
        x_in(c).start()
    for cp in w_in[1:]:
        cp.start()
    _transpose_into(wa, awqkv_v)

    def tok(c):
        return pl.ds(pl.multiple_of(c * T, T), T)

    def a_proj(c, x):
        qkv = _dot(wa[...], _layernorm_t(x))
        pq[:, tok(c)] = _phi(qkv[0:D]).astype(BF16)
        pk[:, tok(c)] = _phi(qkv[D:2 * D]).astype(BF16)
        va[:, tok(c)] = qkv[2 * D:3 * D].astype(BF16)

    def a_state():
        _transpose_into(woa, awo_v)
        _transpose_into(wb, bwqkv_v)
        _transpose_into(wob, bwo_v)
        for j, (lo, hi) in enumerate(BANDS):
            n = hi - lo
            lhs = jnp.concatenate(
                [va[lo:hi, :], jnp.ones((16, S), BF16)], axis=0)
            r = _dot_nt(lhs, pk[j * 128:(j + 1) * 128, :])
            e = lax.broadcasted_iota(jnp.int32, (n, 128), 0) + lo
            d = lax.broadcasted_iota(jnp.int32, (n, 128), 1) + j * 128
            same = _head_of(e) == _head_of(d)
            kvz[j, 0:n, :] = jnp.where(same, r[0:n], 0.0).astype(BF16)
            kvz[j, BAND_MAX:BAND_MAX + n, :] = jnp.where(
                same, r[n:n + 1], 0.0).astype(BF16)

    def band_sum(parts):
        rows = []
        for j, (lo, hi) in enumerate(BANDS):
            own_lo = lo if j == 0 else BANDS[j - 1][1]
            nxt_lo = hi if j == len(BANDS) - 1 else BANDS[j + 1][0]
            rows.append(parts[j][own_lo - lo:nxt_lo - lo])
            if nxt_lo < hi:
                rows.append(parts[j][nxt_lo - lo:hi - lo]
                            + parts[j + 1][0:hi - nxt_lo])
        return jnp.concatenate(rows, axis=0)

    def a_out(c, x):
        nums, dens = [], []
        for j, (lo, hi) in enumerate(BANDS):
            n = hi - lo
            q = pq[j * 128:(j + 1) * 128, tok(c)]
            nums.append(_dot(kvz[j, 0:n, :], q))
            dens.append(_dot(kvz[j, BAND_MAX:BAND_MAX + n, :], q))
        o = band_sum(nums) / (band_sum(dens) + 1e-6)
        return x + _dot(woa[...], o.astype(BF16))

    def b_proj(c, x):
        qkv = _dot(wb[...], _layernorm_t(x))
        q = qkv[0:D] * (DH ** -0.5 * np.log2(np.e))
        for w, lo in enumerate(WIN):
            qw[w, :, tok(c)] = q[lo:lo + 128]
            kw[w, tok(c), :] = qkv[D + lo:D + lo + 128].T.astype(BF16)
        v = qkv[2 * D:3 * D].astype(BF16).astype(F32)
        row = lax.broadcasted_iota(jnp.int32, (VR, T), 0)
        for h in range(H):
            lo = 8 * (DH * h // 8)
            one = (DH * h % 8 + DH) % VR
            vw[h, :, tok(c)] = jnp.where(row == one, 1.0, v[lo:lo + VR])

    nqt = S // NQ
    nsteps = (H // G) * nqt

    def q_masked(st, g):
        h = (st // nqt) * G + g
        w = jnp.minimum(h // 6, NW - 1)
        off = DH * h - jnp.where(w == NW - 1, WIN[-1], 120 * w)
        q = qw[w, :, pl.ds(pl.multiple_of((st % nqt) * NQ, NQ), NQ)]
        row = lax.broadcasted_iota(jnp.int32, (128, NQ), 0)
        keep = (row >= off) & (row < off + DH)
        return w, jnp.where(keep, q, 0.0).astype(BF16)

    def scores(w, qm, keys, s_dst, g, mx):
        s = _dot(kw[w, keys, :], qm)
        s_dst[g, keys, :] = s
        t = jnp.max(s.reshape(-1, 8, NQ), axis=0)
        return t if mx is None else jnp.maximum(mx, t)

    def attn_quad(st, quad, s_cur, s_nxt):
        outs = []
        for i in range(4):
            g = quad * 4 + i
            if s_nxt is not None:
                w, qm = q_masked(st + 1, g)
            m_cur = m_ref[g, 0:1, :]
            acc = mx = None
            for c in range(S // CH):
                keys = pl.ds(c * CH, CH)
                if s_nxt is not None:
                    mx = scores(w, qm, keys, s_nxt, g, mx)
                p = jnp.exp2(s_cur[g, keys, :] - m_cur).astype(BF16)
                r = _dot(vw[(st // nqt) * G + g, :, keys], p)
                acc = r if acc is None else acc + r
            if s_nxt is not None:
                m_ref[g, 0:1, :] = jnp.max(mx, axis=0, keepdims=True)
            one = (DH * i % 8 + DH) % VR
            outs.append(acc * (1.0 / acc[one:one + 1]))
        row = lax.broadcasted_iota(jnp.int32, (8, NQ), 0)
        rows = []
        for i in (0, 2):
            rows += [outs[i][0:16],
                     jnp.where(row < 4, outs[i][16:24], outs[i + 1][0:8]),
                     outs[i + 1][8:24]]
        ot[(st // nqt) * (G // 4) + quad, :,
           pl.ds(pl.multiple_of((st % nqt) * NQ, NQ), NQ)] = (
               jnp.concatenate(rows, axis=0).astype(BF16))

    def attention():
        def head(g, carry):
            w, qm = q_masked(0, g)
            mx = scores(w, qm, pl.ds(0, S), s_a, g, None)
            m_ref[g, 0:1, :] = jnp.max(mx, axis=0, keepdims=True)
            return carry
        lax.fori_loop(0, G, head, 0)

        def body(st, carry):
            for parity, (s_cur, s_nxt) in enumerate(((s_a, s_b), (s_b, s_a))):
                @pl.when(st % 2 == parity)
                def _():
                    for quad in range(G // 4):
                        attn_quad(st, quad, s_cur, s_nxt)
            return carry
        lax.fori_loop(0, nsteps - 1, body, 0)

        def tail(quad, carry):
            attn_quad(nsteps - 1, quad, s_b, None)
            return carry
        lax.fori_loop(0, G // 4, tail, 0)

    def b_out(c, x):
        o = ot[:, :, tok(c)].reshape(D, T)
        return x + _dot(wob[...], o)

    def chunks(fn):
        def body(c, carry):
            fn(c)
            return carry
        lax.fori_loop(0, S // T, body, 0)

    def into_a(i):
        def fn(c):
            @pl.when(i == 0)
            def _():
                x_in(c).wait()
                xt[:, tok(c)] = xio[tok(c), :].astype(F32).T

            @pl.when(i > 0)
            def _():
                xt[:, tok(c)] = b_out(c, xt[:, tok(c)])
            a_proj(c, xt[:, tok(c)])
        return fn

    def a_to_b(c):
        x = a_out(c, xt[:, tok(c)])
        xt[:, tok(c)] = x
        b_proj(c, x)

    def last(c):
        xio[tok(c), :] = b_out(c, xt[:, tok(c)]).T.astype(xio.dtype)
        x_out(c).start()

    def layer_pair(i, carry):
        a_in = into_a(i)
        chunks(a_in)

        @pl.when(i == 0)
        def _():
            for cp in w_in[1:]:
                cp.wait()
        a_state()
        chunks(a_to_b)
        attention()
        return carry
    lax.fori_loop(0, 2, layer_pair, 0)
    chunks(last)
    for c in range(nch):
        x_out(c).wait()


@jax.jit
def pallas_interleave_layers__linear_attn_block__mha_block__prompt_kernel(
    A_x: jax.Array,
    A_wqkv: jax.Array,
    A_wo: jax.Array,
    B_x: jax.Array,
    B_wqkv: jax.Array,
    B_wo: jax.Array,
):
    del B_x
    out = pl.pallas_call(
        _kernel,
        out_shape=jax.ShapeDtypeStruct((S, D), A_x.dtype),
        in_specs=[pl.BlockSpec(memory_space=pl.ANY)] * 5,
        out_specs=pl.BlockSpec(memory_space=pl.ANY),
        scratch_shapes=[
            pltpu.VMEM((S, D), A_x.dtype),
            pltpu.VMEM((D, 3 * D), BF16),
            pltpu.VMEM((D, D), BF16),
            pltpu.VMEM((D, 3 * D), BF16),
            pltpu.VMEM((D, D), BF16),
            pltpu.SemaphoreType.DMA((S // T + 4,)),
            pltpu.VMEM((D, S), F32),
            pltpu.VMEM((3 * D, D), BF16),
            pltpu.VMEM((D, D), BF16),
            pltpu.VMEM((3 * D, D), BF16),
            pltpu.VMEM((D, D), BF16),
            pltpu.VMEM((D, S), BF16),
            pltpu.VMEM((D, S), BF16),
            pltpu.VMEM((D, S), BF16),
            pltpu.VMEM((5, 2 * BAND_MAX, 128), BF16),
            pltpu.VMEM((NW, 128, S), F32),
            pltpu.VMEM((NW, S, 128), BF16),
            pltpu.VMEM((H, VR, S), F32),
            pltpu.VMEM((H // 4, 4 * DH, S), BF16),
            pltpu.VMEM((G, S, NQ), F32),
            pltpu.VMEM((G, S, NQ), F32),
            pltpu.VMEM((G, 8, NQ), F32),
        ],
        compiler_params=pltpu.CompilerParams(
            vmem_limit_bytes=110 * 1024 * 1024),
    )(A_x.reshape(S, D), A_wqkv, A_wo, B_wqkv, B_wo)
    return out.reshape(A_x.shape)
```

```python
import jax
import jax.numpy as jnp
import numpy as np
from jax import lax
import jax.experimental.pallas as pl
import jax.experimental.pallas.tpu as pltpu

S = 2048
D = 640
H = 32
DH = D // H
T = 512
NQ = 256
CH = 128
G = 8
VR = 24
FILL = 2
NW = 6
F32 = jnp.float32
BF16 = jnp.bfloat16

BANDS = ((0, 144), (112, 272), (240, 400), (368, 528), (496, 640))
BAND_MAX = 160
WIN = (0, 120, 240, 360, 480, 512)


def _layernorm_t(x):
    m = jnp.sum(x, axis=0, keepdims=True) * (1.0 / D)
    xc = x - m
    v = jnp.sum(xc * xc, axis=0, keepdims=True) * (1.0 / D)
    return (xc * lax.rsqrt(v + 1e-5)).astype(BF16)


def _head_of(i):
    return (i * 3277) >> 16


def _phi(t):
    return jnp.where(t > 0, t + 1.0, jnp.exp(t)) + 1e-6


def _dot(a, b):
    return lax.dot_general(a, b, (((1,), (0,)), ((), ())),
                           preferred_element_type=F32)


def _dot_nt(a, b):
    return lax.dot_general(a, b, (((1,), (1,)), ((), ())),
                           preferred_element_type=F32)


def _transpose_into(dst, src):
    for j in range(src.shape[1] // 128):
        dst[j * 128:(j + 1) * 128, :] = (
            src[:, j * 128:(j + 1) * 128].astype(F32).T.astype(BF16))


def _kernel(x_hbm, awqkv_hbm, awo_hbm, bwqkv_hbm, bwo_hbm, o_hbm,
            xio, awqkv_v, awo_v, bwqkv_v, bwo_v, sems,
            xt, wa, woa, wb, wob, pq, pk, va, kvz, qw, kw, vw, ot,
            s_a, s_b, m_ref):
    nch = S // T

    def x_in(c):
        rows = pl.ds(pl.multiple_of(c * T, T), T)
        return pltpu.make_async_copy(x_hbm.at[rows], xio.at[rows], sems.at[c])

    def x_out(c):
        rows = pl.ds(pl.multiple_of(c * T, T), T)
        return pltpu.make_async_copy(xio.at[rows], o_hbm.at[rows], sems.at[c])

    w_in = [pltpu.make_async_copy(src, dst, sems.at[nch + i])
            for i, (src, dst) in enumerate((
                (awo_hbm, awo_v), (bwqkv_hbm, bwqkv_v), (bwo_hbm, bwo_v)))]
    thirds = [pl.ds(i * D, D) for i in range(3)]
    wa_in = [pltpu.make_async_copy(awqkv_hbm.at[:, cols], awqkv_v.at[:, cols],
                                   sems.at[nch + 3 + i])
             for i, cols in enumerate(thirds)]

    wa_in[0].start()
    wa_in[1].start()
    wa_in[0].wait()
    wa_in[2].start()
    x_in(0).start()
    _transpose_into(wa.at[thirds[0]], awqkv_v.at[:, thirds[0]])
    wa_in[1].wait()
    _transpose_into(wa.at[thirds[1]], awqkv_v.at[:, thirds[1]])
    wa_in[2].wait()
    for c in range(1, nch):
        x_in(c).start()
    for cp in w_in:
        cp.start()
    _transpose_into(wa.at[thirds[2]], awqkv_v.at[:, thirds[2]])

    def tok(c):
        return pl.ds(pl.multiple_of(c * T, T), T)

    def a_proj(c, x):
        qkv = _dot(wa[...], _layernorm_t(x))
        pq[:, tok(c)] = _phi(qkv[0:D]).astype(BF16)
        pk[:, tok(c)] = _phi(qkv[D:2 * D]).astype(BF16)
        va[:, tok(c)] = qkv[2 * D:3 * D].astype(BF16)

    def a_state():
        _transpose_into(woa, awo_v)
        _transpose_into(wb, bwqkv_v)
        _transpose_into(wob, bwo_v)
        for j, (lo, hi) in enumerate(BANDS):
            n = hi - lo
            lhs = jnp.concatenate(
                [va[lo:hi, :], jnp.ones((16, S), BF16)], axis=0)
            r = _dot_nt(lhs, pk[j * 128:(j + 1) * 128, :])
            e = lax.broadcasted_iota(jnp.int32, (n, 128), 0) + lo
            d = lax.broadcasted_iota(jnp.int32, (n, 128), 1) + j * 128
            same = _head_of(e) == _head_of(d)
            kvz[j, 0:n, :] = jnp.where(same, r[0:n], 0.0).astype(BF16)
            hh = lax.broadcasted_iota(jnp.int32, (H, 128), 0)
            dd = lax.broadcasted_iota(jnp.int32, (H, 128), 1) + j * 128
            kvz[j, n:n + H, :] = jnp.where(
                hh == _head_of(dd), r[n:n + 1], 0.0).astype(BF16)

    def band_sum(parts):
        rows = []
        for j, (lo, hi) in enumerate(BANDS):
            own_lo = lo if j == 0 else BANDS[j - 1][1]
            nxt_lo = hi if j == len(BANDS) - 1 else BANDS[j + 1][0]
            rows.append(parts[j][own_lo - lo:nxt_lo - lo])
            if nxt_lo < hi:
                rows.append(parts[j][nxt_lo - lo:hi - lo]
                            + parts[j + 1][0:hi - nxt_lo])
        return jnp.concatenate(rows, axis=0)

    def a_out(c, x):
        nums, den = [], None
        for j, (lo, hi) in enumerate(BANDS):
            n = hi - lo
            r = _dot(kvz[j, 0:n + H, :], pq[j * 128:(j + 1) * 128, tok(c)])
            nums.append(r[0:n])
            den = r[n:n + H] if den is None else den + r[n:n + H]
        inv = 1.0 / (den + 1e-6)
        row = lax.broadcasted_iota(jnp.int32, (8, T), 0)
        scale = []
        for h in range(0, H, 2):
            ia = jnp.broadcast_to(inv[h:h + 1], (8, T))
            ib = jnp.broadcast_to(inv[h + 1:h + 2], (8, T))
            scale += [ia, ia, jnp.where(row < 4, ia, ib), ib, ib]
        o = band_sum(nums) * jnp.concatenate(scale, axis=0)
        return x + _dot(woa[...], o.astype(BF16))

    def b_proj(c, x):
        qkv = _dot(wb[...], _layernorm_t(x))
        q = qkv[0:D] * (DH ** -0.5 * np.log2(np.e))
        for w, lo in enumerate(WIN):
            qw[w, :, tok(c)] = q[lo:lo + 128]
            kw[w, tok(c), :] = qkv[D + lo:D + lo + 128].T.astype(BF16)
        v = qkv[2 * D:3 * D].astype(BF16).astype(F32)
        row = lax.broadcasted_iota(jnp.int32, (VR, T), 0)
        for h in range(H):
            lo = 8 * (DH * h // 8)
            one = (DH * h % 8 + DH) % VR
            vw[h, :, tok(c)] = jnp.where(row == one, 1.0, v[lo:lo + VR])

    nqt = S // NQ
    nsteps = (H // G) * nqt

    def group(st):
        return st >> (nqt.bit_length() - 1)

    def queries(st):
        return pl.ds(pl.multiple_of((st & (nqt - 1)) * NQ, NQ), NQ)

    def q_masked(st, g):
        h = group(st) * G + g
        w = (h * 43) >> 8
        off = DH * h - jnp.minimum(120 * w, WIN[-1])
        q = qw[w, :, queries(st)]
        row = lax.broadcasted_iota(jnp.int32, (128, NQ), 0)
        keep = (row >= off) & (row < off + DH)
        return w, jnp.where(keep, q, 0.0).astype(BF16)

    def scores(w, qm, keys, s_dst, g, mx):
        s = _dot(kw[w, keys, :], qm)
        s_dst[g, keys, :] = s
        t = jnp.max(s.reshape(-1, 8, NQ), axis=0)
        return t if mx is None else jnp.maximum(mx, t)

    def attn_quad(st, quad, s_cur, s_nxt, filler=None):
        outs = []
        for i in range(4):
            g = quad * 4 + i
            if s_nxt is not None:
                w, qm = q_masked(st + 1, g)
            m_cur = m_ref[g, 0:1, :]
            acc = mx = None
            for c in range(S // CH):
                keys = pl.ds(c * CH, CH)
                if s_nxt is not None:
                    mx = scores(w, qm, keys, s_nxt, g, mx)
                if filler is not None:
                    filler(i, c)
                p = jnp.exp2(s_cur[g, keys, :] - m_cur).astype(BF16)
                r = _dot(vw[group(st) * G + g, :, keys], p)
                acc = r if acc is None else acc + r
            if s_nxt is not None:
                m_ref[g, 0:1, :] = jnp.max(mx, axis=0, keepdims=True)
            one = (DH * i % 8 + DH) % VR
            outs.append(acc * (1.0 / acc[one:one + 1]))
        row = lax.broadcasted_iota(jnp.int32, (8, NQ), 0)
        rows = []
        for i in (0, 2):
            rows += [outs[i][0:16],
                     jnp.where(row < 4, outs[i][16:24], outs[i + 1][0:8]),
                     outs[i + 1][8:24]]
        ot[group(st) * (G // 4) + quad, :, queries(st)] = (
            jnp.concatenate(rows, axis=0).astype(BF16))

    def attention():
        def head(quad, carry):
            for i in range(4):
                g = quad * 4 + i
                w, qm = q_masked(0, g)
                mx = scores(w, qm, pl.ds(0, S), s_a, g, None)
                m_ref[g, 0:1, :] = jnp.max(mx, axis=0, keepdims=True)
            return carry
        lax.fori_loop(0, G // 4, head, 0)

        def body(st, carry):
            for parity, (s_cur, s_nxt) in enumerate(((s_a, s_b), (s_b, s_a))):
                @pl.when((st & 1) == parity)
                def _():
                    for quad in range(G // 4):
                        attn_quad(st, quad, s_cur, s_nxt)
            return carry
        lax.fori_loop(0, nsteps - 1, body, 0)

        def tail(quad, carry):
            n = T // (G // 4)
            cols = pl.ds(pl.multiple_of(quad * n, n), n)
            o = ot[:, :, cols].reshape(D, n)

            def filler(i, c):
                if c % (S // CH // FILL) == 0:
                    m = D // (4 * FILL)
                    rows = pl.ds((i * FILL + c // (S // CH // FILL)) * m, m)
                    xt[rows, cols] = xt[rows, cols] + _dot(wob[rows, :], o)
            attn_quad(nsteps - 1, quad, s_b, None, filler)
            return carry
        lax.fori_loop(0, G // 4, tail, 0)

    def b_out(cols, n):
        return xt[:, cols] + _dot(wob[...], ot[:, :, cols].reshape(D, n))

    def chunks(fn, first=0):
        def body(c, carry):
            fn(c)
            return carry
        lax.fori_loop(first, S // T, body, 0)

    def into_a(i):
        def fn(c):
            @pl.when(i == 0)
            def _():
                x_in(c).wait()
                xt[:, tok(c)] = xio[tok(c), :].astype(F32).T

            @pl.when(jnp.logical_and(i > 0, c > 0))
            def _():
                xt[:, tok(c)] = b_out(tok(c), T)
            a_proj(c, xt[:, tok(c)])
        return fn

    def a_to_b(c):
        x = a_out(c, xt[:, tok(c)])
        xt[:, tok(c)] = x
        b_proj(c, x)

    def last(c):
        xio[tok(c), :] = b_out(tok(c), T).T.astype(xio.dtype)
        x_out(c).start()

    def layer_pair(i, carry):
        a_in = into_a(i)
        chunks(a_in)

        @pl.when(i == 0)
        def _():
            for cp in w_in:
                cp.wait()
        a_state()
        chunks(a_to_b)
        attention()
        return carry
    lax.fori_loop(0, 2, layer_pair, 0)
    xio[tok(0), :] = xt[:, tok(0)].T.astype(xio.dtype)
    x_out(0).start()
    chunks(last, 1)
    for c in range(nch):
        x_out(c).wait()


@jax.jit
def pallas_interleave_layers__linear_attn_block__mha_block__prompt_kernel(
    A_x: jax.Array,
    A_wqkv: jax.Array,
    A_wo: jax.Array,
    B_x: jax.Array,
    B_wqkv: jax.Array,
    B_wo: jax.Array,
):
    del B_x
    out = pl.pallas_call(
        _kernel,
        out_shape=jax.ShapeDtypeStruct((S, D), A_x.dtype),
        in_specs=[pl.BlockSpec(memory_space=pl.ANY)] * 5,
        out_specs=pl.BlockSpec(memory_space=pl.ANY),
        scratch_shapes=[
            pltpu.VMEM((S, D), A_x.dtype),
            pltpu.VMEM((D, 3 * D), BF16),
            pltpu.VMEM((D, D), BF16),
            pltpu.VMEM((D, 3 * D), BF16),
            pltpu.VMEM((D, D), BF16),
            pltpu.SemaphoreType.DMA((S // T + 6,)),
            pltpu.VMEM((D, S), F32),
            pltpu.VMEM((3 * D, D), BF16),
            pltpu.VMEM((D, D), BF16),
            pltpu.VMEM((3 * D, D), BF16),
            pltpu.VMEM((D, D), BF16),
            pltpu.VMEM((D, S), BF16),
            pltpu.VMEM((D, S), BF16),
            pltpu.VMEM((D, S), BF16),
            pltpu.VMEM((5, BAND_MAX + H, 128), BF16),
            pltpu.VMEM((NW, 128, S), F32),
            pltpu.VMEM((NW, S, 128), BF16),
            pltpu.VMEM((H, VR, S), F32),
            pltpu.VMEM((H // 4, 4 * DH, S), BF16),
            pltpu.VMEM((G, S, NQ), F32),
            pltpu.VMEM((G, S, NQ), F32),
            pltpu.VMEM((G, 8, NQ), F32),
        ],
        compiler_params=pltpu.CompilerParams(
            vmem_limit_bytes=110 * 1024 * 1024),
    )(A_x.reshape(S, D), A_wqkv, A_wo, B_wqkv, B_wo)
    return out.reshape(A_x.shape)
```
